```python
import os as _os
_os.environ.setdefault("JAX_PLATFORMS", "cpu")
import jax
import jax.numpy as jnp

def _softmax(x, axis=-1):
    return jax.nn.softmax(x, axis=axis)
def _gelu(x):
    return jax.nn.gelu(x, approximate=True)
def _silu(x):
    return jax.nn.silu(x)
def _sigmoid(x):
    return jax.nn.sigmoid(x)
def _layernorm(x, axis=-1, eps=1e-5):
    m = jnp.mean(x, axis=axis, keepdims=True)
    v = jnp.var(x, axis=axis, keepdims=True)
    return (x - m) / jnp.sqrt(v + eps)
def _scatter_add(tgt, idx, src, axis=0):
    return tgt.at[idx].add(src)
def _segment_sum(src, seg, n):
    return jax.ops.segment_sum(src, seg, n)
class _Rng:
    def __init__(self, key):
        self._k = key
    def _next(self):
        self._k, sub = jax.random.split(self._k)
        return sub
    def normal(self, shape):
        return jax.random.normal(self._next(), shape, dtype=jnp.bfloat16)
    def randint(self, lo, hi, shape):
        return jax.random.randint(self._next(), shape, lo, hi, dtype=jnp.int32)
    def uniform(self, shape, lo=0.0, hi=1.0):
        return jax.random.uniform(self._next(), shape, jnp.bfloat16, lo, hi)
    def permutation(self, n):
        return jax.random.permutation(self._next(), n)


kernel_name = 'gated_mix__ssm_conv_s5__glu_gated_geglu__prompt'

def setup_inputs():
    _rng = _Rng(jax.random.key(int.from_bytes(__import__("os").urandom(4), "little")))
    _w = (lambda a: (lambda t: t.astype(jnp.bfloat16) if jnp.issubdtype(t.dtype, jnp.floating) else t)(jnp.asarray(a)))
    def _A_setup():
        B, S, D = 1, 2048, 1024
        P = D
        Lambda_re = -0.5 * jnp.exp((lambda *s: _rng.normal(s) * 0.4)(P))
        Lambda_im = (lambda *s: _rng.normal(s) * 0.4)(P) * 1.0
        B_re = (lambda *s: _rng.normal(s) * 0.4)(P, D) * (D ** -0.5)
        B_im = (lambda *s: _rng.normal(s) * 0.4)(P, D) * (D ** -0.5)
        C_re = (lambda *s: _rng.normal(s) * 0.4)(D, P) * (P ** -0.5)
        C_im = (lambda *s: _rng.normal(s) * 0.4)(D, P) * (P ** -0.5)
        log_dt = (lambda *s: _rng.normal(s) * 0.4)(P) * 0.3 - 2.0
        Dskip = (lambda *s: _rng.normal(s) * 0.4)(D)
        return {
            "x": _w((lambda *s: _rng.normal(s) * 0.05)(B, S, D)),
            "Lambda_re": _w(Lambda_re),
            "Lambda_im": _w(Lambda_im),
            "B_re": _w(B_re),
            "B_im": _w(B_im),
            "C_re": _w(C_re),
            "C_im": _w(C_im),
            "log_dt": _w(log_dt),
            "Dskip": _w(Dskip),
        }
    _A_in = _A_setup()

    def _B_setup():
        B, S, Dm, Df = 1, 2048, 1024, 3584
        return {
            "x": _w((lambda *s: _rng.normal(s) * 0.05)(B, S, Dm)),
            "w_gate": _w((lambda *s: _rng.normal(s) * 1.6)(Dm, Df) * (Dm ** -0.5)),
            "w_up": _w((lambda *s: _rng.normal(s) * 1.6)(Dm, Df) * (Dm ** -0.5)),
            "w_down": _w((lambda *s: _rng.normal(s) * 1.6)(Df, Dm) * (Df ** -0.5)),
        }
    _B_in = _B_setup()

    return {
        "A_x": _A_in["x"],
        "A_Lambda_re": _A_in["Lambda_re"],
        "A_Lambda_im": _A_in["Lambda_im"],
        "A_B_re": _A_in["B_re"],
        "A_B_im": _A_in["B_im"],
        "A_C_re": _A_in["C_re"],
        "A_C_im": _A_in["C_im"],
        "A_log_dt": _A_in["log_dt"],
        "A_Dskip": _A_in["Dskip"],
        "B_x": _B_in["x"],
        "B_w_gate": _B_in["w_gate"],
        "B_w_up": _B_in["w_up"],
        "B_w_down": _B_in["w_down"],
        "gate_w": _w((lambda *s: _rng.normal(s) * 0.05)(1024) * 16.0),
    }

def reference(A_x, A_Lambda_re, A_Lambda_im, A_B_re, A_B_im, A_C_re, A_C_im, A_log_dt, A_Dskip, B_x, B_w_gate, B_w_up, B_w_down, gate_w):
    def _A_ref(x, Lambda_re, Lambda_im, B_re, B_im, C_re, C_im, log_dt, Dskip):
        Bsz, L, H = x.shape
        Lam = Lambda_re + 1j * Lambda_im
        Bmat = B_re + 1j * B_im
        Cmat = C_re + 1j * C_im
        dt = jnp.exp(log_dt)
        Lam_bar = jnp.exp(dt * Lam)
        B_bar = ((Lam_bar - 1.0) / Lam)[:, None] * Bmat
        Bu = jnp.einsum("bld,pd->blp", x + 0j, B_bar)
        h = jnp.zeros_like(Bu[:, 0, :])
        hs = []
        for t in range(L):
            h = Lam_bar[None, :] * h + Bu[:, t, :]
            hs.append(h)
        hseq = jnp.stack(hs, 1)
        y = 2.0 * jnp.einsum("blp,dp->bld", hseq, Cmat).real + x * Dskip[None, None, :]
        return y

    def _B_ref(x, w_gate, w_up, w_down):
        g = jnp.einsum("bsd,df->bsf", x, w_gate)
        u = jnp.einsum("bsd,df->bsf", x, w_up)
        h = _gelu(g) * u
        return jnp.einsum("bsf,fd->bsd", h, w_down)

    x = A_x
    g = _sigmoid((x * gate_w).sum(-1, keepdims=True))
    a = _A_ref(x, A_Lambda_re, A_Lambda_im, A_B_re, A_B_im, A_C_re, A_C_im, A_log_dt, A_Dskip)
    b = _B_ref(x, B_w_gate, B_w_up, B_w_down)
    return g * a + (1 - g) * b
```

```python
import functools

import jax
import jax.numpy as jnp
import jax.experimental.pallas as pl
import jax.experimental.pallas.tpu as pltpu

PB = 256
FB = 512
_NT = (((1,), (1,)), ((), ()))


def _gelu_tanh(v):
    c = 0.7978845608028654
    return 0.5 * v * (1.0 + jnp.tanh(c * (v + 0.044715 * (v * v * v))))


def _kernel(x_ref, lre_ref, lim_ref, ldt_ref, bre_ref, bim_ref, cre_ref, cim_ref,
            dsk_ref, gw_ref, wg_ref, wu_ref, wd_ref, o_ref,
            hr_ref, hi_ref, accb_ref, *, ns, ng):
    i = pl.program_id(0)
    L = x_ref.shape[0]

    @pl.when(i == 0)
    def _():
        o_ref[...] = jnp.zeros(o_ref.shape, o_ref.dtype)
        accb_ref[...] = jnp.zeros(accb_ref.shape, accb_ref.dtype)

    @pl.when(i < ns)
    def _ssm():
        lre = lre_ref[...].astype(jnp.float32)
        lim = lim_ref[...].astype(jnp.float32)
        dt = jnp.exp(ldt_ref[...].astype(jnp.float32)).astype(jnp.bfloat16).astype(jnp.float32)
        mag = jnp.exp(dt * lre)
        ang = dt * lim
        ar = mag * jnp.cos(ang)
        ai = mag * jnp.sin(ang)
        den = lre * lre + lim * lim
        nr = ar - 1.0
        cr = (nr * lre + ai * lim) / den
        ci = (ai * lre - nr * lim) / den

        x = x_ref[...]
        vr = jax.lax.dot_general(x, bre_ref[...], _NT, preferred_element_type=jnp.float32)
        vi = jax.lax.dot_general(x, bim_ref[...], _NT, preferred_element_type=jnp.float32)
        hr_ref[...] = cr * vr - ci * vi
        hi_ref[...] = cr * vi + ci * vr

        row = jax.lax.broadcasted_iota(jnp.int32, (8, PB), 0)
        pows = []
        pr, pi = ar, ai
        tr = jnp.zeros((8, PB), jnp.float32)
        ti = jnp.zeros((8, PB), jnp.float32)
        for k in range(8):
            pows.append((pr, pi))
            tr = jnp.where(row == k, pr, tr)
            ti = jnp.where(row == k, pi, ti)
            pr, pi = pr * ar - pi * ai, pr * ai + pi * ar
        cds = []
        for d in (1, 2, 4):
            qr, qi = pows[d - 1]
            cds.append((jnp.where(row >= d, qr, 0.0), jnp.where(row >= d, qi, 0.0)))

        def body(g, carry):
            c_r, c_i = carry
            r0 = pl.multiple_of(g * 8, 8)
            hr = hr_ref[pl.ds(r0, 8), :]
            hi = hi_ref[pl.ds(r0, 8), :]
            for (d, (qr, qi)) in zip((1, 2, 4), cds):
                sr = pltpu.roll(hr, d, 0)
                si = pltpu.roll(hi, d, 0)
                hr, hi = hr + (qr * sr - qi * si), hi + (qr * si + qi * sr)
            hr, hi = hr + (tr * c_r - ti * c_i), hi + (tr * c_i + ti * c_r)
            hr_ref[pl.ds(r0, 8), :] = hr
            hi_ref[pl.ds(r0, 8), :] = hi
            return hr[7:8, :], hi[7:8, :]

        z = jnp.zeros((1, PB), jnp.float32)
        jax.lax.fori_loop(0, L // 8, body, (z, z), unroll=4)

        hrb = hr_ref[...].astype(jnp.bfloat16)
        hib = hi_ref[...].astype(jnp.bfloat16)
        y = jax.lax.dot_general(hrb, cre_ref[...], _NT, preferred_element_type=jnp.float32)
        y = y - jax.lax.dot_general(hib, cim_ref[...], _NT, preferred_element_type=jnp.float32)
        o_ref[...] += y

    @pl.when(i >= ns)
    def _glu():
        x = x_ref[...]
        g = jnp.dot(x, wg_ref[...], preferred_element_type=jnp.float32)
        u = jnp.dot(x, wu_ref[...], preferred_element_type=jnp.float32)
        h = (_gelu_tanh(g) * u).astype(jnp.bfloat16)
        accb_ref[...] += jnp.dot(h, wd_ref[...], preferred_element_type=jnp.float32)

    @pl.when(i == ns + ng - 1)
    def _fin():
        xf = x_ref[...].astype(jnp.float32)
        gw = gw_ref[...].astype(jnp.float32)
        prod = (xf * gw).astype(jnp.bfloat16).astype(jnp.float32)
        s = jnp.sum(prod, axis=-1, keepdims=True).astype(jnp.bfloat16).astype(jnp.float32)
        gate = jax.nn.sigmoid(s).astype(jnp.bfloat16).astype(jnp.float32)
        skip = (xf * dsk_ref[...].astype(jnp.float32)).astype(jnp.bfloat16).astype(jnp.float32)
        a = 2.0 * o_ref[...] + skip
        b = accb_ref[...].astype(jnp.bfloat16).astype(jnp.float32)
        omg = (1.0 - gate).astype(jnp.bfloat16).astype(jnp.float32)
        o_ref[...] = gate * a + (omg * b).astype(jnp.bfloat16).astype(jnp.float32)


@jax.jit
def pallas_gated_mix__ssm_conv_s5__glu_gated_geglu__prompt_kernel(
    A_x: jax.Array,
    A_Lambda_re: jax.Array,
    A_Lambda_im: jax.Array,
    A_B_re: jax.Array,
    A_B_im: jax.Array,
    A_C_re: jax.Array,
    A_C_im: jax.Array,
    A_log_dt: jax.Array,
    A_Dskip: jax.Array,
    B_x: jax.Array,
    B_w_gate: jax.Array,
    B_w_up: jax.Array,
    B_w_down: jax.Array,
    gate_w: jax.Array,
):
    Bsz, L, D = A_x.shape
    P = A_Lambda_re.shape[0]
    F = B_w_gate.shape[1]
    assert Bsz == 1 and P % PB == 0 and F % FB == 0
    ns, ng = P // PB, F // FB

    x2 = A_x.reshape(L, D)
    row = lambda a: a.reshape(1, -1)

    s_idx = lambda i: jnp.minimum(i, ns - 1)
    g_idx = lambda i: jnp.maximum(i - ns, 0)

    in_specs = [
        pl.BlockSpec((L, D), lambda i: (0, 0)),
        pl.BlockSpec((1, PB), lambda i: (0, s_idx(i))),
        pl.BlockSpec((1, PB), lambda i: (0, s_idx(i))),
        pl.BlockSpec((1, PB), lambda i: (0, s_idx(i))),
        pl.BlockSpec((PB, D), lambda i: (s_idx(i), 0)),
        pl.BlockSpec((PB, D), lambda i: (s_idx(i), 0)),
        pl.BlockSpec((D, PB), lambda i: (0, s_idx(i))),
        pl.BlockSpec((D, PB), lambda i: (0, s_idx(i))),
        pl.BlockSpec((1, D), lambda i: (0, 0)),
        pl.BlockSpec((1, D), lambda i: (0, 0)),
        pl.BlockSpec((D, FB), lambda i: (0, g_idx(i))),
        pl.BlockSpec((D, FB), lambda i: (0, g_idx(i))),
        pl.BlockSpec((FB, D), lambda i: (g_idx(i), 0)),
    ]
    out = pl.pallas_call(
        functools.partial(_kernel, ns=ns, ng=ng),
        grid=(ns + ng,),
        in_specs=in_specs,
        out_specs=pl.BlockSpec((L, D), lambda i: (0, 0)),
        out_shape=jax.ShapeDtypeStruct((L, D), jnp.float32),
        scratch_shapes=[
            pltpu.VMEM((L, PB), jnp.float32),
            pltpu.VMEM((L, PB), jnp.float32),
            pltpu.VMEM((L, D), jnp.float32),
        ],
        compiler_params=pltpu.CompilerParams(
            dimension_semantics=("arbitrary",),
            vmem_limit_bytes=100 * 1024 * 1024,
        ),
    )(x2, row(A_Lambda_re), row(A_Lambda_im), row(A_log_dt), A_B_re, A_B_im,
      A_C_re, A_C_im, row(A_Dskip), row(gate_w), B_w_gate, B_w_up, B_w_down)
    return out.reshape(Bsz, L, D)
```

```python
import functools

import jax
import jax.numpy as jnp
import jax.experimental.pallas as pl
import jax.experimental.pallas.tpu as pltpu

PB = 256
FB = 512
TM = 256
_NT = (((1,), (1,)), ((), ()))
_F32 = jnp.float32
_BF16 = jnp.bfloat16


def _gelu_tanh(v):
    c = 0.7978845608028654
    return 0.5 * v * (1.0 + jnp.tanh(c * (v + 0.044715 * (v * v * v))))


def _rb(v):
    return v.astype(_BF16).astype(_F32)


def _kernel(lre_ref, lim_ref, ldt_ref, dsk_ref, gw_ref,
            x_hbm, bre_hbm, bim_hbm, cre_hbm, cim_hbm, wg_hbm, wu_hbm, wd_hbm,
            o_hbm,
            x_v, bre_v, bim_v, cre_v, cim_v, wg_v, wu_v, wd_v,
            hr_v, hi_v, acc_v, tab_v, ost_v,
            x_sem, b_sem, c_sem, g_sem, o_sem):
    L, D = x_v.shape
    P = bre_v.shape[0]
    F = wd_v.shape[0]
    nch, ns, ng = L // TM, P // PB, F // FB

    def x_cp(c):
        return pltpu.make_async_copy(x_hbm.at[pl.ds(c * TM, TM)], x_v.at[pl.ds(c * TM, TM)], x_sem.at[c])

    def b_cp(k, s):
        src, dst = ((bre_hbm, bre_v), (bim_hbm, bim_v))[k]
        return pltpu.make_async_copy(src.at[pl.ds(s * PB, PB)], dst.at[pl.ds(s * PB, PB)], b_sem.at[k, s])

    def c_cp(k):
        src, dst = ((cre_hbm, cre_v), (cim_hbm, cim_v))[k]
        return pltpu.make_async_copy(src, dst, c_sem.at[k])

    def g_cp(k, j):
        if k == 2:
            return pltpu.make_async_copy(wd_hbm.at[pl.ds(j * FB, FB)], wd_v.at[pl.ds(j * FB, FB)], g_sem.at[2, j])
        src, dst = ((wg_hbm, wg_v), (wu_hbm, wu_v))[k]
        return pltpu.make_async_copy(src.at[:, pl.ds(j * FB, FB)], dst.at[:, pl.ds(j * FB, FB)], g_sem.at[k, j])

    def o_cp(slot, c):
        return pltpu.make_async_copy(ost_v.at[slot], o_hbm.at[pl.ds(c * TM, TM)], o_sem.at[slot])

    x_cp(0).start()
    b_cp(0, 0).start()
    b_cp(1, 0).start()
    for c in range(1, nch):
        x_cp(c).start()
    for s in range(1, ns):
        b_cp(0, s).start()
        b_cp(1, s).start()

    lre = lre_ref[...].astype(_F32)
    lim = lim_ref[...].astype(_F32)
    dt = _rb(jnp.exp(ldt_ref[...].astype(_F32)))
    mag = jnp.exp(dt * lre)
    ang = dt * lim
    ar = mag * jnp.cos(ang)
    ai = mag * jnp.sin(ang)
    den = lre * lre + lim * lim
    nr = ar - 1.0
    cr = (nr * lre + ai * lim) / den
    ci = (ai * lre - nr * lim) / den
    row = jax.lax.broadcasted_iota(jnp.int32, (8, P), 0)
    pows = []
    pr, pi = ar, ai
    tr = jnp.zeros((8, P), _F32)
    ti = jnp.zeros((8, P), _F32)
    for k in range(8):
        pows.append((pr, pi))
        tr = jnp.where(row == k, pr, tr)
        ti = jnp.where(row == k, pi, ti)
        pr, pi = pr * ar - pi * ai, pr * ai + pi * ar
    tab_v[0] = tr
    tab_v[1] = ti
    for n, d in enumerate((1, 2, 4)):
        qr, qi = pows[d - 1]
        tab_v[2 + 2 * n] = jnp.where(row >= d, qr, 0.0)
        tab_v[3 + 2 * n] = jnp.where(row >= d, qi, 0.0)
    tab_v[8] = jnp.broadcast_to(cr, (8, P))
    tab_v[9] = jnp.broadcast_to(ci, (8, P))

    def a_body(it, _):
        s = it // nch
        c = it % nch
        r0 = pl.multiple_of(c * TM, TM)
        p0 = pl.multiple_of(s * PB, PB)

        @pl.when(s == 0)
        def _():
            x_cp(c).wait()

        @pl.when(c == 0)
        def _():
            b_cp(0, s).wait()
            b_cp(1, s).wait()
            for k in range(3):
                g_cp(k, s).start()

        x = x_v[pl.ds(r0, TM), :]
        vr = jax.lax.dot_general(x, bre_v[pl.ds(p0, PB), :], _NT, preferred_element_type=_F32)
        vi = jax.lax.dot_general(x, bim_v[pl.ds(p0, PB), :], _NT, preferred_element_type=_F32)
        kr = tab_v[8, 0:1, pl.ds(p0, PB)]
        ki = tab_v[9, 0:1, pl.ds(p0, PB)]
        hr_v[pl.ds(r0, TM), pl.ds(p0, PB)] = kr * vr - ki * vi
        hi_v[pl.ds(r0, TM), pl.ds(p0, PB)] = kr * vi + ki * vr
        return 0

    jax.lax.fori_loop(0, ns * nch, a_body, 0)

    def glu_item(j, c):
        r0 = pl.multiple_of(c * TM, TM)
        f0 = pl.multiple_of(j * FB, FB)
        x = x_v[pl.ds(r0, TM), :]
        g = jnp.dot(x, wg_v[:, pl.ds(f0, FB)], preferred_element_type=_F32)
        u = jnp.dot(x, wu_v[:, pl.ds(f0, FB)], preferred_element_type=_F32)
        h = (_gelu_tanh(g) * u).astype(_BF16)
        d = jnp.dot(h, wd_v[pl.ds(f0, FB), :], preferred_element_type=_F32)
        prev = acc_v[pl.ds(r0, TM), :]
        acc_v[pl.ds(r0, TM), :] = jnp.where(j == 0, d, prev + d)

    def glu_waits(j, c):
        @pl.when(c == 0)
        def _():
            for k in range(3):
                g_cp(k, j).wait()

            @pl.when(j + ns < ng)
            def _():
                for k in range(3):
                    g_cp(k, j + ns).start()

            @pl.when(j == 0)
            def _():
                c_cp(0).start()
                c_cp(1).start()

    def scan_item(s, c, carry):
        p0 = pl.multiple_of(s * PB, PB)
        tr = tab_v[0, :, pl.ds(p0, PB)]
        ti = tab_v[1, :, pl.ds(p0, PB)]
        cds = [(tab_v[2 + 2 * n, :, pl.ds(p0, PB)], tab_v[3 + 2 * n, :, pl.ds(p0, PB)]) for n in range(3)]
        c_r = jnp.where(c == 0, 0.0, carry[0])
        c_i = jnp.where(c == 0, 0.0, carry[1])
        for g in range(TM // 8):
            r0 = pl.multiple_of(c * TM + g * 8, 8)
            hr = hr_v[pl.ds(r0, 8), pl.ds(p0, PB)]
            hi = hi_v[pl.ds(r0, 8), pl.ds(p0, PB)]
            for (d, (qr, qi)) in zip((1, 2, 4), cds):
                sr = pltpu.roll(hr, d, 0)
                si = pltpu.roll(hi, d, 0)
                hr, hi = hr + (qr * sr - qi * si), hi + (qr * si + qi * sr)
            hr, hi = hr + (tr * c_r - ti * c_i), hi + (tr * c_i + ti * c_r)
            hr_v[pl.ds(r0, 8), pl.ds(p0, PB)] = hr
            hi_v[pl.ds(r0, 8), pl.ds(p0, PB)] = hi
            c_r, c_i = hr[7:8, :], hi[7:8, :]
        return c_r, c_i

    def b1_body(it, carry):
        j = it // nch
        c = it % nch
        glu_waits(j, c)
        carry = scan_item(j, c, carry)
        glu_item(j, c)
        return carry

    z = jnp.zeros((1, PB), _F32)
    jax.lax.fori_loop(0, ns * nch, b1_body, (z, z))

    def b2_body(it, _):
        j = it // nch
        c = it % nch
        glu_waits(j, c)
        glu_item(j, c)
        return 0

    jax.lax.fori_loop(ns * nch, ng * nch, b2_body, 0)

    c_cp(0).wait()
    c_cp(1).wait()
    gw = gw_ref[...].astype(_F32)
    dsk = dsk_ref[...].astype(_F32)

    def c_body(c, _):
        r0 = pl.multiple_of(c * TM, TM)
        slot = c % 2

        @pl.when(c >= 2)
        def _():
            o_cp(slot, c - 2).wait()

        hrb = hr_v[pl.ds(r0, TM), :].astype(_BF16)
        hib = hi_v[pl.ds(r0, TM), :].astype(_BF16)
        y = jax.lax.dot_general(hrb, cre_v[...], _NT, preferred_element_type=_F32)
        y = y - jax.lax.dot_general(hib, cim_v[...], _NT, preferred_element_type=_F32)
        xf = x_v[pl.ds(r0, TM), :].astype(_F32)
        s = _rb(jnp.sum(_rb(xf * gw), axis=-1, keepdims=True))
        gate = _rb(jax.nn.sigmoid(s))
        a = 2.0 * y + _rb(xf * dsk)
        b = _rb(acc_v[pl.ds(r0, TM), :])
        ost_v[slot] = gate * a + _rb(_rb(1.0 - gate) * b)
        o_cp(slot, c).start()
        return 0

    jax.lax.fori_loop(0, nch, c_body, 0)
    o_cp(0, nch - 2).wait()
    o_cp(1, nch - 1).wait()


@jax.jit
def pallas_gated_mix__ssm_conv_s5__glu_gated_geglu__prompt_kernel(
    A_x: jax.Array,
    A_Lambda_re: jax.Array,
    A_Lambda_im: jax.Array,
    A_B_re: jax.Array,
    A_B_im: jax.Array,
    A_C_re: jax.Array,
    A_C_im: jax.Array,
    A_log_dt: jax.Array,
    A_Dskip: jax.Array,
    B_x: jax.Array,
    B_w_gate: jax.Array,
    B_w_up: jax.Array,
    B_w_down: jax.Array,
    gate_w: jax.Array,
):
    Bsz, L, D = A_x.shape
    P = A_Lambda_re.shape[0]
    F = B_w_gate.shape[1]
    assert Bsz == 1 and P % PB == 0 and F % FB == 0 and L % (2 * TM) == 0
    assert F // FB >= P // PB
    nch, ns, ng = L // TM, P // PB, F // FB

    x2 = A_x.reshape(L, D)
    row = lambda a: a.reshape(1, -1)
    vm = pl.BlockSpec(memory_space=pltpu.VMEM)
    hbm = pl.BlockSpec(memory_space=pl.ANY)

    out = pl.pallas_call(
        _kernel,
        in_specs=[vm] * 5 + [hbm] * 8,
        out_specs=hbm,
        out_shape=jax.ShapeDtypeStruct((L, D), _F32),
        scratch_shapes=[
            pltpu.VMEM((L, D), _BF16),
            pltpu.VMEM((P, D), _BF16),
            pltpu.VMEM((P, D), _BF16),
            pltpu.VMEM((D, P), _BF16),
            pltpu.VMEM((D, P), _BF16),
            pltpu.VMEM((D, F), _BF16),
            pltpu.VMEM((D, F), _BF16),
            pltpu.VMEM((F, D), _BF16),
            pltpu.VMEM((L, P), _F32),
            pltpu.VMEM((L, P), _F32),
            pltpu.VMEM((L, D), _F32),
            pltpu.VMEM((10, 8, P), _F32),
            pltpu.VMEM((2, TM, D), _F32),
            pltpu.SemaphoreType.DMA((nch,)),
            pltpu.SemaphoreType.DMA((2, ns)),
            pltpu.SemaphoreType.DMA((2,)),
            pltpu.SemaphoreType.DMA((3, ng)),
            pltpu.SemaphoreType.DMA((2,)),
        ],
        compiler_params=pltpu.CompilerParams(
            vmem_limit_bytes=110 * 1024 * 1024,
        ),
    )(row(A_Lambda_re), row(A_Lambda_im), row(A_log_dt), row(A_Dskip), row(gate_w),
      x2, A_B_re, A_B_im, A_C_re, A_C_im, B_w_gate, B_w_up, B_w_down)
    return out.reshape(Bsz, L, D)
```

```python
import jax
import jax.numpy as jnp
import jax.experimental.pallas as pl
import jax.experimental.pallas.tpu as pltpu

PB = 256
FB = 896
TA = 256
TA2 = 2048
TB = 1024
TC = 256
_NT = (((1,), (1,)), ((), ()))
_F32 = jnp.float32
_BF16 = jnp.bfloat16


def _rb(v):
    return v.astype(_BF16).astype(_F32)


def _gelu_tanh(v):
    c = 0.7978845608028654
    return 0.5 * v * (1.0 + jnp.tanh(c * (v + 0.044715 * (v * v * v))))


def _kernel(lre_ref, lim_ref, ldt_ref, dsk_ref, gw_ref,
            x_hbm, bre_hbm, bim_hbm, cre_hbm, cim_hbm, wg_hbm, wu_hbm, wd_hbm,
            o_hbm,
            x_v, bre_v, bim_v, cre_v, cim_v, wg_v, wu_v, wd_v,
            hr_v, hi_v, acc_v, tab_v, ost_v,
            x_sem, b_sem, c_sem, g_sem, o_sem):
    L, D = x_v.shape
    P = bre_v.shape[0]
    F = wd_v.shape[0]
    ns, ng = P // PB, F // FB
    na, na2, nb, nc = L // TA, L // TA2, L // TB, L // TC

    def x_cp(c):
        return pltpu.make_async_copy(x_hbm.at[pl.ds(c * TA, TA)], x_v.at[pl.ds(c * TA, TA)], x_sem.at[c])

    def b_cp(k, s):
        src, dst = ((bre_hbm, bre_v), (bim_hbm, bim_v))[k]
        return pltpu.make_async_copy(src.at[pl.ds(s * PB, PB)], dst.at[pl.ds(s * PB, PB)], b_sem.at[k, s])

    def c_cp(k):
        src, dst = ((cre_hbm, cre_v), (cim_hbm, cim_v))[k]
        return pltpu.make_async_copy(src, dst, c_sem.at[k])

    def g_cp(k, j):
        if k == 2:
            return pltpu.make_async_copy(wd_hbm.at[pl.ds(j * FB, FB)], wd_v.at[pl.ds(j * FB, FB)], g_sem.at[2, j])
        src, dst = ((wg_hbm, wg_v), (wu_hbm, wu_v))[k]
        return pltpu.make_async_copy(src.at[:, pl.ds(j * FB, FB)], dst.at[:, pl.ds(j * FB, FB)], g_sem.at[k, j])

    def o_cp(q):
        return pltpu.make_async_copy(ost_v.at[pl.ds(q * TC, TC)], o_hbm.at[pl.ds(q * TC, TC)], o_sem.at[q])

    x_cp(0).start()
    b_cp(0, 0).start()
    b_cp(1, 0).start()
    for c in range(1, na):
        x_cp(c).start()
    for s in range(1, ns):
        b_cp(0, s).start()
        b_cp(1, s).start()

    lre = lre_ref[...].astype(_F32).reshape(1, P)
    lim = lim_ref[...].astype(_F32).reshape(1, P)
    dt = _rb(jnp.exp(ldt_ref[...].astype(_F32).reshape(1, P)))
    mag = jnp.exp(dt * lre)
    ang = dt * lim
    ar = mag * jnp.cos(ang)
    ai = mag * jnp.sin(ang)
    den = lre * lre + lim * lim
    nr = ar - 1.0
    cr = (nr * lre + ai * lim) / den
    ci = (ai * lre - nr * lim) / den
    row = jax.lax.broadcasted_iota(jnp.int32, (8, P), 0)
    pows = []
    pr, pi = ar, ai
    tr = jnp.zeros((8, P), _F32)
    ti = jnp.zeros((8, P), _F32)
    for k in range(8):
        pows.append((pr, pi))
        tr = jnp.where(row == k, pr, tr)
        ti = jnp.where(row == k, pi, ti)
        pr, pi = pr * ar - pi * ai, pr * ai + pi * ar
    tab_v[0] = tr
    tab_v[1] = ti
    for n, d in enumerate((1, 2, 4)):
        qr, qi = pows[d - 1]
        tab_v[2 + 2 * n] = jnp.where(row >= d, qr, 0.0)
        tab_v[3 + 2 * n] = jnp.where(row >= d, qi, 0.0)
    tab_v[8] = jnp.broadcast_to(cr, (8, P))
    tab_v[9] = jnp.broadcast_to(ci, (8, P))

    def a_item(s, r0, rows):
        p0 = pl.multiple_of(s * PB, PB)
        x = x_v[pl.ds(r0, rows), :]
        vr = jax.lax.dot_general(x, bre_v[pl.ds(p0, PB), :], _NT, preferred_element_type=_F32)
        vi = jax.lax.dot_general(x, bim_v[pl.ds(p0, PB), :], _NT, preferred_element_type=_F32)
        kr = tab_v[8, 0:1, pl.ds(p0, PB)]
        ki = tab_v[9, 0:1, pl.ds(p0, PB)]
        hr_v[pl.ds(r0, rows), pl.ds(p0, PB)] = kr * vr - ki * vi
        hi_v[pl.ds(r0, rows), pl.ds(p0, PB)] = kr * vi + ki * vr

    b_cp(0, 0).wait()
    b_cp(1, 0).wait()
    for k in range(3):
        g_cp(k, 0).start()

    def a1_body(c, _):
        x_cp(c).wait()
        a_item(0, pl.multiple_of(c * TA, TA), TA)
        return 0

    jax.lax.fori_loop(0, na, a1_body, 0)

    def a2_body(it, _):
        s = 1 + it // na2
        c = it % na2

        @pl.when(c == 0)
        def _():
            b_cp(0, s).wait()
            b_cp(1, s).wait()
            for k in range(3):
                g_cp(k, s).start()

        a_item(s, pl.multiple_of(c * TA2, TA2), TA2)
        return 0

    jax.lax.fori_loop(0, (ns - 1) * na2, a2_body, 0)

    def glu_item(j, c):
        r0 = pl.multiple_of(c * TB, TB)
        f0 = pl.multiple_of(j * FB, FB)
        x = x_v[pl.ds(r0, TB), :]
        g = jnp.dot(x, wg_v[:, pl.ds(f0, FB)], preferred_element_type=_F32)
        u = jnp.dot(x, wu_v[:, pl.ds(f0, FB)], preferred_element_type=_F32)
        h = (_gelu_tanh(g) * u).astype(_BF16)
        d = jnp.dot(h, wd_v[pl.ds(f0, FB), :], preferred_element_type=_F32)
        prev = acc_v[pl.ds(r0, TB), :]
        acc_v[pl.ds(r0, TB), :] = jnp.where(j == 0, d, prev + d)

    def glu_waits(j, c):
        @pl.when(c == 0)
        def _():
            for k in range(3):
                g_cp(k, j).wait()

            if ng > ns:
                @pl.when(j + ns < ng)
                def _():
                    for k in range(3):
                        g_cp(k, j + ns).start()

            @pl.when(j == 0)
            def _():
                c_cp(0).start()
                c_cp(1).start()

    def scan_item(s, c, carry):
        p0 = pl.multiple_of(s * PB, PB)
        tr = tab_v[0, :, pl.ds(p0, PB)]
        ti = tab_v[1, :, pl.ds(p0, PB)]
        cds = [(tab_v[2 + 2 * n, :, pl.ds(p0, PB)], tab_v[3 + 2 * n, :, pl.ds(p0, PB)]) for n in range(3)]
        c_r = jnp.where(c == 0, 0.0, carry[0])
        c_i = jnp.where(c == 0, 0.0, carry[1])
        for g in range(TB // 8):
            r0 = pl.multiple_of(c * TB + g * 8, 8)
            hr = hr_v[pl.ds(r0, 8), pl.ds(p0, PB)]
            hi = hi_v[pl.ds(r0, 8), pl.ds(p0, PB)]
            for (d, (qr, qi)) in zip((1, 2, 4), cds):
                sr = pltpu.roll(hr, d, 0)
                si = pltpu.roll(hi, d, 0)
                hr, hi = hr + (qr * sr - qi * si), hi + (qr * si + qi * sr)
            hr, hi = hr + (tr * c_r - ti * c_i), hi + (tr * c_i + ti * c_r)
            hr_v[pl.ds(r0, 8), pl.ds(p0, PB)] = hr
            hi_v[pl.ds(r0, 8), pl.ds(p0, PB)] = hi
            c_r, c_i = hr[7:8, :], hi[7:8, :]
        return c_r, c_i

    def b1_body(it, carry):
        j = it // nb
        c = it % nb
        glu_waits(j, c)
        carry = scan_item(j, c, carry)
        glu_item(j, c)
        return carry

    z = jnp.zeros((1, PB), _F32)
    jax.lax.fori_loop(0, ns * nb, b1_body, (z, z))

    if ng > ns:
        def b2_body(it, _):
            j = it // nb
            c = it % nb
            glu_waits(j, c)
            glu_item(j, c)
            return 0

        jax.lax.fori_loop(ns * nb, ng * nb, b2_body, 0)

    c_cp(0).wait()
    c_cp(1).wait()
    gw = gw_ref[...].astype(_F32).reshape(1, D)
    dsk = dsk_ref[...].astype(_F32).reshape(1, D)

    def c_body(c, _):
        r0 = pl.multiple_of(c * TC, TC)
        hrb = hr_v[pl.ds(r0, TC), :].astype(_BF16)
        hib = hi_v[pl.ds(r0, TC), :].astype(_BF16)
        y = jax.lax.dot_general(hrb, cre_v[...], _NT, preferred_element_type=_F32)
        y = y - jax.lax.dot_general(hib, cim_v[...], _NT, preferred_element_type=_F32)
        xf = x_v[pl.ds(r0, TC), :].astype(_F32)
        s = _rb(jnp.sum(_rb(xf * gw), axis=-1, keepdims=True))
        gate = _rb(jax.nn.sigmoid(s))
        a = 2.0 * y + _rb(xf * dsk)
        b = _rb(acc_v[pl.ds(r0, TC), :])
        ost_v[pl.ds(r0, TC), :] = gate * a + _rb(_rb(1.0 - gate) * b)
        o_cp(c).start()
        return 0

    jax.lax.fori_loop(0, nc, c_body, 0)
    for q in range(nc):
        o_cp(q).wait()


@jax.jit
def pallas_gated_mix__ssm_conv_s5__glu_gated_geglu__prompt_kernel(
    A_x: jax.Array,
    A_Lambda_re: jax.Array,
    A_Lambda_im: jax.Array,
    A_B_re: jax.Array,
    A_B_im: jax.Array,
    A_C_re: jax.Array,
    A_C_im: jax.Array,
    A_log_dt: jax.Array,
    A_Dskip: jax.Array,
    B_x: jax.Array,
    B_w_gate: jax.Array,
    B_w_up: jax.Array,
    B_w_down: jax.Array,
    gate_w: jax.Array,
):
    Bsz, L, D = A_x.shape
    P = A_Lambda_re.shape[0]
    F = B_w_gate.shape[1]
    assert Bsz == 1 and P % PB == 0 and F % FB == 0
    assert L % TA == 0 and L % TA2 == 0 and L % TB == 0 and L % TC == 0
    assert F // FB >= P // PB
    ns, ng = P // PB, F // FB

    vm = pl.BlockSpec(memory_space=pltpu.VMEM)
    hbm = pl.BlockSpec(memory_space=pl.ANY)

    out = pl.pallas_call(
        _kernel,
        in_specs=[vm] * 5 + [hbm] * 8,
        out_specs=hbm,
        out_shape=jax.ShapeDtypeStruct((L, D), _F32),
        scratch_shapes=[
            pltpu.VMEM((L, D), _BF16),
            pltpu.VMEM((P, D), _BF16),
            pltpu.VMEM((P, D), _BF16),
            pltpu.VMEM((D, P), _BF16),
            pltpu.VMEM((D, P), _BF16),
            pltpu.VMEM((D, F), _BF16),
            pltpu.VMEM((D, F), _BF16),
            pltpu.VMEM((F, D), _BF16),
            pltpu.VMEM((L, P), _F32),
            pltpu.VMEM((L, P), _F32),
            pltpu.VMEM((L, D), _F32),
            pltpu.VMEM((10, 8, P), _F32),
            pltpu.VMEM((L, D), _F32),
            pltpu.SemaphoreType.DMA((L // TA,)),
            pltpu.SemaphoreType.DMA((2, ns)),
            pltpu.SemaphoreType.DMA((2,)),
            pltpu.SemaphoreType.DMA((3, ng)),
            pltpu.SemaphoreType.DMA((L // TC,)),
        ],
        compiler_params=pltpu.CompilerParams(
            vmem_limit_bytes=110 * 1024 * 1024,
        ),
    )(A_Lambda_re, A_Lambda_im, A_log_dt, A_Dskip, gate_w,
      A_x.reshape(L, D), A_B_re, A_B_im, A_C_re, A_C_im, B_w_gate, B_w_up, B_w_down)
    return out.reshape(Bsz, L, D)
```

```python
import jax
import jax.numpy as jnp
import jax.experimental.pallas as pl
import jax.experimental.pallas.tpu as pltpu

PB = 256
FB = 896
TA = 256
TA2 = 2048
TB = 1024
TC = 256
_NT = (((1,), (1,)), ((), ()))
_F32 = jnp.float32
_BF16 = jnp.bfloat16


def _rb(v):
    return v.astype(_BF16).astype(_F32)


def _gelu_tanh(v):
    c = 0.7978845608028654
    return 0.5 * v * (1.0 + jnp.tanh(c * (v + 0.044715 * (v * v * v))))


def _kernel(lre_ref, lim_ref, ldt_ref, dsk_ref, gw_ref,
            x_hbm, bre_hbm, bim_hbm, cre_hbm, cim_hbm, wg_hbm, wu_hbm, wd_hbm,
            o_hbm,
            x_v, bre_v, bim_v, cre_v, cim_v, wg_v, wu_v, wd_v,
            hr_v, hi_v, acc_v, tab_v, ost_v,
            x_sem, b_sem, c_sem, g_sem, o_sem):
    L, D = x_v.shape
    P = bre_v.shape[0]
    F = wd_v.shape[0]
    ns, ng = P // PB, F // FB
    na, na2, nb, nc = L // TA, L // TA2, L // TB, L // TC

    def x_cp(c):
        return pltpu.make_async_copy(x_hbm.at[pl.ds(c * TA, TA)], x_v.at[pl.ds(c * TA, TA)], x_sem.at[c])

    def b_cp(k, s):
        src, dst = ((bre_hbm, bre_v), (bim_hbm, bim_v))[k]
        return pltpu.make_async_copy(src.at[pl.ds(s * PB, PB)], dst.at[pl.ds(s * PB, PB)], b_sem.at[k, s])

    def c_cp(k):
        src, dst = ((cre_hbm, cre_v), (cim_hbm, cim_v))[k]
        return pltpu.make_async_copy(src, dst, c_sem.at[k])

    def g_cp(k, j):
        if k == 2:
            return pltpu.make_async_copy(wd_hbm.at[pl.ds(j * FB, FB)], wd_v.at[pl.ds(j * FB, FB)], g_sem.at[2, j])
        src, dst = ((wg_hbm, wg_v), (wu_hbm, wu_v))[k]
        return pltpu.make_async_copy(src.at[:, pl.ds(j * FB, FB)], dst.at[:, pl.ds(j * FB, FB)], g_sem.at[k, j])

    def o_cp(q):
        return pltpu.make_async_copy(ost_v.at[pl.ds(q * TC, TC)], o_hbm.at[pl.ds(q * TC, TC)], o_sem.at[q])

    x_cp(0).start()
    b_cp(0, 0).start()
    b_cp(1, 0).start()
    for c in range(1, na):
        x_cp(c).start()
    for s in range(1, ns):
        b_cp(0, s).start()
        b_cp(1, s).start()

    def z_body(c, _):
        acc_v[pl.ds(pl.multiple_of(c * TC, TC), TC), :] = jnp.zeros((TC, D), _F32)
        return 0

    jax.lax.fori_loop(0, nc, z_body, 0)

    lre = lre_ref[...].astype(_F32).reshape(1, P)
    lim = lim_ref[...].astype(_F32).reshape(1, P)
    dt = _rb(jnp.exp(ldt_ref[...].astype(_F32).reshape(1, P)))
    mag = jnp.exp(dt * lre)
    ang = dt * lim
    ar = mag * jnp.cos(ang)
    ai = mag * jnp.sin(ang)
    den = lre * lre + lim * lim
    nr = ar - 1.0
    cr = (nr * lre + ai * lim) / den
    ci = (ai * lre - nr * lim) / den
    row = jax.lax.broadcasted_iota(jnp.int32, (8, P), 0)
    pows = []
    pr, pi = ar, ai
    tr = jnp.zeros((8, P), _F32)
    ti = jnp.zeros((8, P), _F32)
    for k in range(8):
        pows.append((pr, pi))
        tr = jnp.where(row == k, pr, tr)
        ti = jnp.where(row == k, pi, ti)
        pr, pi = pr * ar - pi * ai, pr * ai + pi * ar
    tab_v[0] = tr
    tab_v[1] = ti
    for n, d in enumerate((1, 2, 4)):
        qr, qi = pows[d - 1]
        tab_v[2 + 2 * n] = jnp.where(row >= d, qr, 0.0)
        tab_v[3 + 2 * n] = jnp.where(row >= d, qi, 0.0)
    tab_v[8] = jnp.broadcast_to(cr, (8, P))
    tab_v[9] = jnp.broadcast_to(ci, (8, P))

    def a_item(s, r0, rows):
        p0 = pl.multiple_of(s * PB, PB)
        x = x_v[pl.ds(r0, rows), :]
        vr = jax.lax.dot_general(x, bre_v[pl.ds(p0, PB), :], _NT, preferred_element_type=_F32)
        vi = jax.lax.dot_general(x, bim_v[pl.ds(p0, PB), :], _NT, preferred_element_type=_F32)
        kr = tab_v[8, 0:1, pl.ds(p0, PB)]
        ki = tab_v[9, 0:1, pl.ds(p0, PB)]
        hr_v[pl.ds(r0, rows), pl.ds(p0, PB)] = kr * vr - ki * vi
        hi_v[pl.ds(r0, rows), pl.ds(p0, PB)] = kr * vi + ki * vr

    b_cp(0, 0).wait()
    b_cp(1, 0).wait()
    for k in range(3):
        g_cp(k, 0).start()

    def a1_body(c, _):
        x_cp(c).wait()
        a_item(0, pl.multiple_of(c * TA, TA), TA)
        return 0

    jax.lax.fori_loop(0, na, a1_body, 0)

    def a2_body(it, _):
        s = 1 + it // na2
        c = it % na2

        @pl.when(c == 0)
        def _():
            b_cp(0, s).wait()
            b_cp(1, s).wait()
            for k in range(3):
                g_cp(k, s).start()

        a_item(s, pl.multiple_of(c * TA2, TA2), TA2)
        return 0

    jax.lax.fori_loop(0, (ns - 1) * na2, a2_body, 0)

    def glu_item(j, c):
        r0 = pl.multiple_of(c * TB, TB)
        f0 = pl.multiple_of(j * FB, FB)
        x = x_v[pl.ds(r0, TB), :]
        g = jnp.dot(x, wg_v[:, pl.ds(f0, FB)], preferred_element_type=_F32)
        u = jnp.dot(x, wu_v[:, pl.ds(f0, FB)], preferred_element_type=_F32)
        h = (_gelu_tanh(g) * u).astype(_BF16)
        d = jnp.dot(h, wd_v[pl.ds(f0, FB), :], preferred_element_type=_F32)
        acc_v[pl.ds(r0, TB), :] += d

    def glu_waits(j, c):
        @pl.when(c == 0)
        def _():
            for k in range(3):
                g_cp(k, j).wait()

            if ng > ns:
                @pl.when(j + ns < ng)
                def _():
                    for k in range(3):
                        g_cp(k, j + ns).start()

            @pl.when(j == 0)
            def _():
                c_cp(0).start()
                c_cp(1).start()

    def scan_item(s, c, carry):
        p0 = pl.multiple_of(s * PB, PB)
        tr = tab_v[0, :, pl.ds(p0, PB)]
        ti = tab_v[1, :, pl.ds(p0, PB)]
        cds = [(tab_v[2 + 2 * n, :, pl.ds(p0, PB)], tab_v[3 + 2 * n, :, pl.ds(p0, PB)]) for n in range(3)]
        c_r = jnp.where(c == 0, 0.0, carry[0])
        c_i = jnp.where(c == 0, 0.0, carry[1])
        for g in range(TB // 8):
            r0 = pl.multiple_of(c * TB + g * 8, 8)
            hr = hr_v[pl.ds(r0, 8), pl.ds(p0, PB)]
            hi = hi_v[pl.ds(r0, 8), pl.ds(p0, PB)]
            for (d, (qr, qi)) in zip((1, 2, 4), cds):
                sr = pltpu.roll(hr, d, 0)
                si = pltpu.roll(hi, d, 0)
                hr, hi = hr + (qr * sr - qi * si), hi + (qr * si + qi * sr)
            hr, hi = hr + (tr * c_r - ti * c_i), hi + (tr * c_i + ti * c_r)
            hr_v[pl.ds(r0, 8), pl.ds(p0, PB)] = hr
            hi_v[pl.ds(r0, 8), pl.ds(p0, PB)] = hi
            c_r, c_i = hr[7:8, :], hi[7:8, :]
        return c_r, c_i

    def b1_body(it, carry):
        j = it // nb
        c = it % nb
        glu_waits(j, c)
        carry = scan_item(j, c, carry)
        glu_item(j, c)
        return carry

    z = jnp.zeros((1, PB), _F32)
    jax.lax.fori_loop(0, ns * nb, b1_body, (z, z))

    if ng > ns:
        def b2_body(it, _):
            j = it // nb
            c = it % nb
            glu_waits(j, c)
            glu_item(j, c)
            return 0

        jax.lax.fori_loop(ns * nb, ng * nb, b2_body, 0)

    c_cp(0).wait()
    c_cp(1).wait()
    gw = gw_ref[...].astype(_F32).reshape(1, D)
    dsk = dsk_ref[...].astype(_F32).reshape(1, D)

    def c_body(c, _):
        r0 = pl.multiple_of(c * TC, TC)
        hrb = hr_v[pl.ds(r0, TC), :].astype(_BF16)
        hib = hi_v[pl.ds(r0, TC), :].astype(_BF16)
        y = jax.lax.dot_general(hrb, cre_v[...], _NT, preferred_element_type=_F32)
        y = y - jax.lax.dot_general(hib, cim_v[...], _NT, preferred_element_type=_F32)
        xf = x_v[pl.ds(r0, TC), :].astype(_F32)
        s = _rb(jnp.sum(_rb(xf * gw), axis=-1, keepdims=True))
        gate = _rb(jax.nn.sigmoid(s))
        a = 2.0 * y + _rb(xf * dsk)
        b = _rb(acc_v[pl.ds(r0, TC), :])
        ost_v[pl.ds(r0, TC), :] = gate * a + _rb(_rb(1.0 - gate) * b)
        o_cp(c).start()
        return 0

    jax.lax.fori_loop(0, nc, c_body, 0)
    for q in range(nc):
        o_cp(q).wait()


@jax.jit
def pallas_gated_mix__ssm_conv_s5__glu_gated_geglu__prompt_kernel(
    A_x: jax.Array,
    A_Lambda_re: jax.Array,
    A_Lambda_im: jax.Array,
    A_B_re: jax.Array,
    A_B_im: jax.Array,
    A_C_re: jax.Array,
    A_C_im: jax.Array,
    A_log_dt: jax.Array,
    A_Dskip: jax.Array,
    B_x: jax.Array,
    B_w_gate: jax.Array,
    B_w_up: jax.Array,
    B_w_down: jax.Array,
    gate_w: jax.Array,
):
    Bsz, L, D = A_x.shape
    P = A_Lambda_re.shape[0]
    F = B_w_gate.shape[1]
    assert Bsz == 1 and P % PB == 0 and F % FB == 0
    assert L % TA == 0 and L % TA2 == 0 and L % TB == 0 and L % TC == 0
    assert F // FB >= P // PB
    ns, ng = P // PB, F // FB

    vm = pl.BlockSpec(memory_space=pltpu.VMEM)
    hbm = pl.BlockSpec(memory_space=pl.ANY)

    out = pl.pallas_call(
        _kernel,
        in_specs=[vm] * 5 + [hbm] * 8,
        out_specs=hbm,
        out_shape=jax.ShapeDtypeStruct((L, D), _F32),
        scratch_shapes=[
            pltpu.VMEM((L, D), _BF16),
            pltpu.VMEM((P, D), _BF16),
            pltpu.VMEM((P, D), _BF16),
            pltpu.VMEM((D, P), _BF16),
            pltpu.VMEM((D, P), _BF16),
            pltpu.VMEM((D, F), _BF16),
            pltpu.VMEM((D, F), _BF16),
            pltpu.VMEM((F, D), _BF16),
            pltpu.VMEM((L, P), _F32),
            pltpu.VMEM((L, P), _F32),
            pltpu.VMEM((L, D), _F32),
            pltpu.VMEM((10, 8, P), _F32),
            pltpu.VMEM((L, D), _F32),
            pltpu.SemaphoreType.DMA((L // TA,)),
            pltpu.SemaphoreType.DMA((2, ns)),
            pltpu.SemaphoreType.DMA((2,)),
            pltpu.SemaphoreType.DMA((3, ng)),
            pltpu.SemaphoreType.DMA((L // TC,)),
        ],
        compiler_params=pltpu.CompilerParams(
            vmem_limit_bytes=110 * 1024 * 1024,
        ),
    )(A_Lambda_re, A_Lambda_im, A_log_dt, A_Dskip, gate_w,
      A_x.reshape(L, D), A_B_re, A_B_im, A_C_re, A_C_im, B_w_gate, B_w_up, B_w_down)
    return out.reshape(Bsz, L, D)
```
